```python
import os as _os
_os.environ.setdefault("JAX_PLATFORMS", "cpu")
import jax
import jax.numpy as jnp

def _softmax(x, axis=-1):
    return jax.nn.softmax(x, axis=axis)
def _gelu(x):
    return jax.nn.gelu(x, approximate=True)
def _silu(x):
    return jax.nn.silu(x)
def _sigmoid(x):
    return jax.nn.sigmoid(x)
def _layernorm(x, axis=-1, eps=1e-5):
    m = jnp.mean(x, axis=axis, keepdims=True)
    v = jnp.var(x, axis=axis, keepdims=True)
    return (x - m) / jnp.sqrt(v + eps)
def _scatter_add(tgt, idx, src, axis=0):
    return tgt.at[idx].add(src)
def _segment_sum(src, seg, n):
    return jax.ops.segment_sum(src, seg, n)
class _Rng:
    def __init__(self, key):
        self._k = key
    def _next(self):
        self._k, sub = jax.random.split(self._k)
        return sub
    def normal(self, shape):
        return jax.random.normal(self._next(), shape, dtype=jnp.bfloat16)
    def randint(self, lo, hi, shape):
        return jax.random.randint(self._next(), shape, lo, hi, dtype=jnp.int32)
    def uniform(self, shape, lo=0.0, hi=1.0):
        return jax.random.uniform(self._next(), shape, jnp.bfloat16, lo, hi)
    def permutation(self, n):
        return jax.random.permutation(self._next(), n)


kernel_name = 'sequential_preLN__mha_block__mixer_token_mlp__prompt'

def setup_inputs():
    _rng = _Rng(jax.random.key(int.from_bytes(__import__("os").urandom(4), "little")))
    _w = (lambda a: (lambda t: t.astype(jnp.bfloat16) if jnp.issubdtype(t.dtype, jnp.floating) else t)(jnp.asarray(a)))
    def _A_setup():
        B, S, D, H = 1, 2048, 448, 16
        return {
            "x": _w((lambda *s: _rng.normal(s) * 0.05)(B, S, D)),
            "wqkv": _w((lambda *s: _rng.normal(s) * 0.05)(D, 3 * D)),
            "wo": _w((lambda *s: _rng.normal(s) * 0.05)(D, D)),
        }
    _A_in = _A_setup()

    def _B_setup():
        B, S, D, F = 1, 2048, 448, 1792
        return {
            "x": _w((lambda *s: _rng.normal(s) * 0.05)(B, S, D)),
            "w1": _w((lambda *s: _rng.normal(s) * 0.2)(S, F) * (S ** -0.5)),
            "b1": _w((lambda *s: _rng.normal(s) * 0.2)(F) * 0.02),
            "w2": _w((lambda *s: _rng.normal(s) * 0.2)(F, S) * (F ** -0.5)),
            "b2": _w((lambda *s: _rng.normal(s) * 0.05)(S) * 0.02),
        }
    _B_in = _B_setup()

    return {
        "A_x": _A_in["x"],
        "A_wqkv": _A_in["wqkv"],
        "A_wo": _A_in["wo"],
        "B_x": _B_in["x"],
        "B_w1": _B_in["w1"],
        "B_b1": _B_in["b1"],
        "B_w2": _B_in["w2"],
        "B_b2": _B_in["b2"],
    }

def reference(A_x, A_wqkv, A_wo, B_x, B_w1, B_b1, B_w2, B_b2):
    def _A_ref(x, wqkv, wo):
        B, S, D = x.shape
        H = 16
        Dh = D // H
        qkv = (lambda x, *d: x.transpose(*d))((x @ wqkv).reshape(B, S, 3, H, Dh), 2, 0, 3, 1, 4)
        q, k, v = qkv[0], qkv[1], qkv[2]
        scores = jnp.einsum("bhqd,bhkd->bhqk", q, k) * (Dh ** -0.5)
        p = _softmax(scores, axis=-1)
        o = jnp.einsum("bhqk,bhkd->bhqd", p, v)
        return (lambda x, *d: x.transpose(*d))(o, 0, 2, 1, 3).reshape(B, S, D) @ wo

    def _B_ref(x, w1, b1, w2, b2):
        B, S, D = x.shape
        h = _layernorm(x, axis=-1)
        u = jnp.einsum("bsd,sf->bdf", h, w1) + b1
        u = _gelu(u)
        y = jnp.einsum("bdf,fs->bds", u, w2) + b2
        return (lambda x, *d: x.transpose(*d))(y, 0, 2, 1)

    x = A_x
    h = x + _A_ref(_layernorm(x, axis=-1), A_wqkv, A_wo)
    h2 = h + _B_ref(_layernorm(h, axis=-1), B_w1, B_b1, B_w2, B_b2)
    return h2
```

```python
import jax
import jax.numpy as jnp
import jax.experimental.pallas as pl
import jax.experimental.pallas.tpu as pltpu

S, D, H, F = 2048, 448, 16, 1792
DH = D // H
HP = 32
DP = H * HP
BQ = 512
CK = 256
LA = 1
RC = 16
WC = (0, 256, 512, 896, 1344)
NW = 2
FC = (0, 512, 896)
OC = (0, 512, 896, 1024)
DEN_LO, DEN_HI = 2.0 ** -40, 2.0 ** 16
F32, BF16 = jnp.float32, jnp.bfloat16


def _ln_stats(load):
    def total(f):
        acc = sum(f(load(r)).reshape(RC // 8, 8, BQ).sum(axis=0) for r in range(0, D, RC))
        return jnp.sum(acc, axis=0, keepdims=True) / D

    m = total(lambda x: x)
    v = total(lambda x: (x - m) * (x - m))
    return m, 1.0 / jnp.sqrt(v + 1e-5)


def _one_row(h):
    return DH if h % 2 == 0 else 0


def _pad_heads(w):
    zer = jnp.zeros((HP - DH, w.shape[1]), F32)
    parts = []
    for h in range(H):
        wh = w[h * DH:(h + 1) * DH]
        parts += [wh, zer] if h % 2 == 0 else [zer, wh]
    return jnp.concatenate(parts, axis=0)


def _store_lhs(l_ref, cols, a11, a12, a21, a22):
    for i, a in enumerate((a11 + a22, a21 + a22, a11, a22, a11 + a12, a21 - a11, a12 - a22)):
        l_ref[i, :, cols] = a.astype(BF16)


def _strassen(l_ref, w_ref, c1, c2):
    k = w_ref.shape[0] // 2

    def w(r, c):
        return w_ref[r * k:(r + 1) * k, c2 if c else c1]

    def mm(i, b):
        return jnp.dot(l_ref[i], b.astype(BF16), preferred_element_type=F32)

    def wf(r, c):
        return w(r, c).astype(F32)

    m2 = mm(1, w(0, 0))
    m5 = mm(4, w(1, 1))
    m1 = mm(0, wf(0, 0) + wf(1, 1))
    m3 = mm(2, wf(0, 1) - wf(1, 1))
    m4 = mm(3, wf(1, 0) - wf(0, 0))
    m6 = mm(5, wf(0, 0) + wf(0, 1))
    m7 = mm(6, wf(1, 0) + wf(1, 1))
    return m1 + m4 - m5 + m7, m3 + m5, m2 + m4, m1 - m2 + m3 + m6


def _kernel(x_hbm, wqkv_hbm, wo_hbm, w1_hbm, b1_hbm, w2_hbm, b2_hbm, o_hbm,
            x_ref, wqkv_ref, wo_ref, w1_ref, b1_ref, w2_ref, b2_ref, o_ref, sems,
            xn_ref, wt_ref, wot_ref, t_ref, kn_ref, q_ref, k_ref, v_ref, a_ref,
            qs_ref, p_ref, h_ref, l1_ref, l2_ref):
    nj = S // BQ
    wcols = list(zip(WC[:-1], WC[1:]))
    cx = [pltpu.make_async_copy(x_hbm.at[:, j * BQ:(j + 1) * BQ], x_ref.at[:, j * BQ:(j + 1) * BQ],
                                sems.at[j]) for j in range(nj)]
    cw = [pltpu.make_async_copy(wqkv_hbm.at[:, lo:hi], wqkv_ref.at[:, lo:hi], sems.at[nj + t])
          for t, (lo, hi) in enumerate(wcols)]
    late = [pltpu.make_async_copy(src, dst, sems.at[nj + len(wcols) + t]) for t, (src, dst) in enumerate(
        [(b1_hbm, b1_ref), (b2_hbm, b2_ref), (w1_hbm, w1_ref), (w2_hbm, w2_ref)])]
    co = pltpu.make_async_copy(wo_hbm, wo_ref, sems.at[nj + len(wcols) + len(late)])
    first = cw[:NW] + [cx[0]]
    for c in first:
        c.start()

    scale = (DH ** -0.5) * 1.4426950408889634
    hrow = jax.lax.broadcasted_iota(jnp.int32, (HP, BQ), 0)

    def ln1(j):
        sl = slice(j * BQ, (j + 1) * BQ)
        m, rs = _ln_stats(lambda r: x_ref[r:r + RC, sl].astype(F32))
        for r in range(0, D, RC):
            xn_ref[r:r + RC, sl] = ((x_ref[r:r + RC, sl].astype(F32) - m) * rs).astype(BF16)

    def wt(i):
        lo, hi = wcols[i]
        wt_ref[lo:hi, :] = wqkv_ref[:, lo:hi].T

    for c in first:
        c.wait()
    for c in cw[NW:] + cx[1:2]:
        c.start()
    wt(0)
    ln1(0)

    def mm(j, lo, hi):
        t_ref[j, lo:hi, :] = jnp.dot(wt_ref[lo:hi, :], xn_ref[:, j * BQ:(j + 1) * BQ],
                                     preferred_element_type=F32)

    def qkv(j):
        for i, (lo, hi) in enumerate(wcols):
            mm(j, lo, hi)
            if i == 0 and j + 1 < nj:
                ln1(j + 1)

    for i in range(NW):
        if i:
            wt(i)
        mm(0, *wcols[i])
    for c in cw[NW:]:
        c.wait()
    for c in cx[2:] + [co]:
        c.start()
    for i in range(NW, len(wcols)):
        wt(i)
    for i in range(NW, len(wcols) - 1):
        mm(0, *wcols[i])
    cx[1].wait()
    ln1(1)
    mm(0, *wcols[-1])
    for c in cx[2:] + [co]:
        c.wait()
    for c in late:
        c.start()

    def window(j, part, h):
        lo = h * DH // 8 * 8
        own = (hrow >= h * DH - lo) & (hrow < (h + 1) * DH - lo)
        return t_ref[j, part * D + lo:part * D + lo + HP, :], own

    lane = jax.lax.broadcasted_iota(jnp.int32, (BQ, HP), 1)
    for j in range(nj):
        sl = slice(j * BQ, (j + 1) * BQ)
        if j + 1 < nj:
            qkv(j + 1)
        for h in range(H):
            hs = slice(h * HP, (h + 1) * HP)
            q, own = window(j, 0, h)
            q = jnp.where(own, q * scale, 0.0)
            qn = jnp.sqrt(jnp.sum(q * q, axis=0, keepdims=True))
            q_ref[j, hs, :] = jnp.where(hrow == _one_row(h), qn, q).astype(BF16)
            k, own = window(j, 1, h)
            kn = jnp.sum(jnp.where(own, k * k, 0.0), axis=0, keepdims=True)
            kn_ref[h] = jnp.broadcast_to(kn, (8, BQ)) if j == 0 else jnp.maximum(kn_ref[h], kn)
            v, _ = window(j, 2, h)
            v_ref[hs, sl] = jnp.where(hrow == _one_row(h), 1.0, v).astype(BF16)
        for g in range(H // 4):
            kt = t_ref[j, D + g * 4 * DH:D + g * 4 * DH + 128, :].astype(BF16).T
            for i in range(4):
                k = kt[:, i * DH // 8 * 8:i * DH // 8 * 8 + HP]
                k_ref[4 * g + i, sl, :] = jnp.where(lane == _one_row(i), jnp.ones_like(k), k)

    wot_ref[...] = _pad_heads(wo_ref[...].astype(F32)).T.astype(BF16)

    def k_max(h):
        return jnp.sqrt(jnp.max(kn_ref[h][0:1], axis=1, keepdims=True))

    def head_q(h, j, kmax):
        q = q_ref[j, pl.ds(pl.multiple_of(h * HP, HP), HP), :].astype(F32)
        spare = hrow == jnp.where(h % 2 == 0, _one_row(0), _one_row(1))
        if kmax is None:
            return jnp.where(spare, 0.0, q).astype(BF16)
        return (q * jnp.where(spare, -kmax, 1.0)).astype(BF16)

    nc = S // CK

    def pv(h, c, p):
        hs = pl.ds(pl.multiple_of(h * HP, HP), HP)
        return jnp.dot(v_ref[hs, c * CK:(c + 1) * CK], p, preferred_element_type=F32)

    def denom(h, acc):
        return jnp.where(h % 2 == 0, acc[_one_row(0):_one_row(0) + 1], acc[_one_row(1):_one_row(1) + 1])

    def finish(h, j, acc, bad):
        den = denom(h, acc)
        a_ref[j, pl.ds(pl.multiple_of((h + 1) * HP, HP), HP), :] = (acc * (1.0 / den)).astype(BF16)
        return jnp.maximum(bad, jnp.where((den >= DEN_LO) & (den <= DEN_HI), 0.0, 1.0))

    def fast(h, carry):
        bad, acc = carry
        hn = jnp.minimum(h + 1, H - 1)
        kmax = k_max(hn)
        n_items = nj * nc
        pend = []
        for n in range(n_items):
            j, c = divmod(n, nc)
            if c == 0:
                qm = qs_ref[j]
            s = jnp.dot(k_ref[h, c * CK:(c + 1) * CK, :], qm, preferred_element_type=F32)
            pend.append(jnp.exp2(s).astype(BF16))
            if c == 1:
                qs_ref[j] = head_q(hn, j, kmax)
            if n == 0:
                bad = finish(h - 1, nj - 1, acc + pv(jnp.maximum(h - 1, 0), nc - 1, p_ref[...]), bad)
            todo = range(n - LA, n - LA + 1) if n + 1 < n_items else range(n - LA, n)
            for i in todo:
                if i >= 0:
                    j, c = divmod(i, nc)
                    r = pv(h, c, pend.pop(0))
                    acc = r if c == 0 else acc + r
                    if c == nc - 1:
                        bad = finish(h, j, acc, bad)
        p_ref[...] = pend.pop(0)
        return bad, acc

    kmax = k_max(0)
    for j in range(nj):
        qs_ref[j] = head_q(0, j, kmax)
    p_ref[...] = jnp.zeros((CK, BQ), BF16)
    bad, acc = jax.lax.fori_loop(0, H, fast, (jnp.zeros((1, BQ), F32), jnp.ones((HP, BQ), F32)))
    bad = finish(H - 1, nj - 1, acc + pv(H - 1, nc - 1, p_ref[...]), bad)

    @pl.when(jnp.max(bad) > 0.0)
    def _():
        def safe(i, carry):
            h, j = i // nj, i % nj
            hs = pl.ds(pl.multiple_of(h * HP, HP), HP)
            s = jnp.dot(k_ref[h], head_q(h, j, None), preferred_element_type=F32)
            p = jnp.exp2(s - jnp.max(s, axis=0, keepdims=True)).astype(BF16)
            acc = jnp.dot(v_ref[hs, :], p, preferred_element_type=F32)
            a_ref[j, pl.ds(pl.multiple_of((h + 1) * HP, HP), HP), :] = (acc / denom(h, acc)).astype(BF16)
            return carry

        jax.lax.fori_loop(0, H * nj, safe, 0)

    for c in late:
        c.wait()

    def ln2(j):
        sl = slice(j * BQ, (j + 1) * BQ)
        h_ref[:, sl] = x_ref[:, sl].astype(F32) + jnp.dot(
            wot_ref[...], a_ref[j, HP:, :], preferred_element_type=F32)
        m, rs = _ln_stats(lambda r: h_ref[r:r + RC, sl])
        return lambda r: (h_ref[r:r + RC, sl] - m) * rs

    for j in range(nj // 2):
        lo, hi = ln2(j), ln2(j + nj // 2)
        for r in range(0, D // 2, RC):
            _store_lhs(l1_ref.at[:, r:r + RC], slice(j * BQ, (j + 1) * BQ),
                       lo(r), hi(r), lo(D // 2 + r), hi(D // 2 + r))

    b1 = b1_ref[...].astype(F32).reshape(1, F)
    b2 = b2_ref[...].astype(F32).reshape(1, S)
    for lo, hi in zip(FC[:-1], FC[1:]):
        c1, c2 = slice(lo, hi), slice(F // 2 + lo, F // 2 + hi)
        u11, u12, u21, u22 = _strassen(l1_ref, w1_ref, c1, c2)
        _store_lhs(l2_ref, c1, *[jax.nn.gelu(u + b1[:, c], approximate=True)
                                 for u, c in ((u11, c1), (u12, c2), (u21, c1), (u22, c2))])
    outs = []
    top, bot = slice(0, D // 2), slice(D // 2, D)
    for lo, hi in zip(OC[:-1], OC[1:]):
        c1, c2 = slice(lo, hi), slice(S // 2 + lo, S // 2 + hi)
        for y, r, c in zip(_strassen(l2_ref, w2_ref, c1, c2), (top, top, bot, bot), (c1, c2, c1, c2)):
            o_ref[r, c] = (y + b2[:, c] + h_ref[r, c]).astype(BF16)
        for c in (c1, c2):
            outs.append(pltpu.make_async_copy(o_ref.at[:, c], o_hbm.at[:, c], sems.at[len(outs)]))
            outs[-1].start()
    for c in outs:
        c.wait()


@jax.jit
def pallas_sequential_preLN__mha_block__mixer_token_mlp__prompt_kernel(
    A_x, A_wqkv, A_wo, B_x, B_w1, B_b1, B_w2, B_b2
):
    del B_x
    hbm = pl.BlockSpec(memory_space=pl.ANY)
    out = pl.pallas_call(
        _kernel,
        out_shape=jax.ShapeDtypeStruct((D, S), BF16),
        in_specs=[hbm] * 7,
        out_specs=hbm,
        scratch_shapes=[
            pltpu.VMEM((D, S), BF16),
            pltpu.VMEM((D, 3 * D), BF16),
            pltpu.VMEM((D, D), BF16),
            pltpu.VMEM((S, F), BF16),
            pltpu.VMEM((F,), BF16),
            pltpu.VMEM((F, S), BF16),
            pltpu.VMEM((S,), BF16),
            pltpu.VMEM((D, S), BF16),
            pltpu.SemaphoreType.DMA((32,)),
            pltpu.VMEM((D, S), BF16),
            pltpu.VMEM((3 * D, D), BF16),
            pltpu.VMEM((D, DP), BF16),
            pltpu.VMEM((S // BQ, 3 * D, BQ), F32),
            pltpu.VMEM((H, 8, BQ), F32),
            pltpu.VMEM((S // BQ, DP, BQ), BF16),
            pltpu.VMEM((H, S, HP), BF16),
            pltpu.VMEM((DP, S), BF16),
            pltpu.VMEM((S // BQ, DP + HP, BQ), BF16),
            pltpu.VMEM((S // BQ, HP, BQ), BF16),
            pltpu.VMEM((CK, BQ), BF16),
            pltpu.VMEM((D, S), F32),
            pltpu.VMEM((7, D // 2, S // 2), BF16),
            pltpu.VMEM((7, D // 2, F // 2), BF16),
        ],
        compiler_params=pltpu.CompilerParams(vmem_limit_bytes=100 * 1024 * 1024),
    )(A_x.reshape(S, D).T, A_wqkv, A_wo, B_w1, B_b1, B_w2, B_b2)
    return out.T.reshape(1, S, D)
```
